```python
import jax
import jax.numpy as jnp

def _softmax(x, axis=-1):
    return jax.nn.softmax(x, axis=axis)
def _gelu(x):
    return jax.nn.gelu(x, approximate=True)
def _silu(x):
    return jax.nn.silu(x)
def _sigmoid(x):
    return jax.nn.sigmoid(x)
def _layernorm(x, axis=-1, eps=1e-5):
    m = jnp.mean(x, axis=axis, keepdims=True)
    v = jnp.var(x, axis=axis, keepdims=True)
    return (x - m) / jnp.sqrt(v + eps)
def _scatter_add(tgt, idx, src, axis=0):
    return tgt.at[idx].add(src)
def _segment_sum(src, seg, n):
    return jax.ops.segment_sum(src, seg, n)
class _Rng:
    def __init__(self, key):
        self._k = key
    def _next(self):
        self._k, sub = jax.random.split(self._k)
        return sub
    def normal(self, shape):
        return jax.random.normal(self._next(), shape, dtype=jnp.bfloat16)
    def randint(self, lo, hi, shape):
        return jax.random.randint(self._next(), shape, lo, hi, dtype=jnp.int32)
    def uniform(self, shape, lo=0.0, hi=1.0):
        return jax.random.uniform(self._next(), shape, jnp.bfloat16, lo, hi)
    def permutation(self, n):
        return jax.random.permutation(self._next(), n)


kernel_name = 'gated_mix__sliding_block_cached__moe_arch_mod__decode'

def setup_inputs():
    _rng = _Rng(jax.random.key(int.from_bytes(__import__("os").urandom(4), "little")))
    _w = (lambda a: (lambda t: t.astype(jnp.bfloat16) if jnp.issubdtype(t.dtype, jnp.floating) else t)(jnp.asarray(a)))
    def _A_setup():
        B, Sq, D = 1, 1, 640
        Hq, Hkv, Sk, Dh = 32, 32, 32768, 192
        assert Hq % Hkv == 0, (Hq, Hkv)
        return {
            "x": _w((lambda *s: _rng.normal(s) * 0.05)(B, Sq, D)),
            "k_cache": _w((lambda *s: _rng.normal(s) * 0.05)(B, Hkv, Sk, Dh)),
            "v_cache": _w((lambda *s: _rng.normal(s) * 0.05)(B, Hkv, Sk, Dh)),
            "wq": _w((lambda *s: _rng.normal(s) * 0.05)(D, Hq * Dh) * (D ** -0.5)),
            "wo": _w((lambda *s: _rng.normal(s) * 0.05)(Hq * Dh, D) * ((Hq * Dh) ** -0.5)),
        }
    _A_in = _A_setup()

    def _B_setup():
        B, S, D, F, C = 1, 1, 640, 1536, 1
        return {
            "x": _w((lambda *s: _rng.normal(s) * 0.05)(B, S, D)),
            "w_r": _w((lambda *s: _rng.normal(s) * 0.05)(D)),
            "w_gate": _w((lambda *s: _rng.normal(s) * 0.05)(D, F)),
            "w_up": _w((lambda *s: _rng.normal(s) * 0.05)(D, F)),
            "w_down": _w((lambda *s: _rng.normal(s) * 0.05)(F, D)),
        }
    _B_in = _B_setup()

    return {
        "A_x": _A_in["x"],
        "A_k_cache": _A_in["k_cache"],
        "A_v_cache": _A_in["v_cache"],
        "A_wq": _A_in["wq"],
        "A_wo": _A_in["wo"],
        "B_x": _B_in["x"],
        "B_w_r": _B_in["w_r"],
        "B_w_gate": _B_in["w_gate"],
        "B_w_up": _B_in["w_up"],
        "B_w_down": _B_in["w_down"],
        "gate_w": _w((lambda *s: _rng.normal(s) * 0.05)(640)),
    }

def reference(A_x, A_k_cache, A_v_cache, A_wq, A_wo, B_x, B_w_r, B_w_gate, B_w_up, B_w_down, gate_w):
    def _A_ref(x, k_cache, v_cache, wq, wo):
        B, Sq, D = x.shape
        Hq, Dh = 32, 192
        Hkv, Sk = k_cache.shape[1], k_cache.shape[2]
        W = min(4096, max(256, Sk // 4))
        rep = Hq // Hkv
        q = (lambda x, *d: x.transpose(*d))((x @ wq).reshape(B, Sq, Hq, Dh), 0, 2, 1, 3)
        k = jnp.repeat(k_cache[:, :, Sk - W:, :], rep, axis=1)
        v = jnp.repeat(v_cache[:, :, Sk - W:, :], rep, axis=1)
        scores = jnp.einsum("bhqd,bhkd->bhqk", q, k) * (Dh ** -0.5)
        p = _softmax(scores, axis=-1)
        o = jnp.einsum("bhqk,bhkd->bhqd", p, v)
        return (lambda x, *d: x.transpose(*d))(o, 0, 2, 1, 3).reshape(B, Sq, Hq * Dh) @ wo

    def _B_ref(x, w_r, w_gate, w_up, w_down):
        B, S, D = x.shape
        C = 1
        r = x @ w_r
        idx = jnp.argsort(-r, axis=-1)[:, :C]
        idx_e = jnp.repeat(idx.reshape(B, C, 1), D, axis=2)
        x_sel = jnp.take_along_axis(x, idx_e, axis=1)
        g = _silu(x_sel @ w_gate)
        u = x_sel @ w_up
        y = (g * u) @ w_down
        r_sel = _sigmoid(jnp.take_along_axis(r, idx, axis=1))
        y = y * r_sel.reshape(B, C, 1)
        b_off = (jnp.arange(B) * S).reshape(B, 1)
        flat_idx = (idx + b_off).reshape(B * C)
        zero = (x * 0.0).reshape(B * S, D)
        upd = _scatter_add(zero, flat_idx, y.reshape(B * C, D), axis=0)
        return x + upd.reshape(B, S, D)

    x = A_x
    g = _sigmoid((x * gate_w).sum(-1, keepdims=True))
    a = _A_ref(x, A_k_cache, A_v_cache, A_wq, A_wo)
    b = _B_ref(x, B_w_r, B_w_gate, B_w_up, B_w_down)
    return g * a + (1 - g) * b
```

```python
import functools
import jax
import jax.numpy as jnp
import jax.experimental.pallas as pl
import jax.experimental.pallas.tpu as pltpu

H, DH, SK, WIN, D, F = 32, 192, 32768, 4096, 640, 1536
f32, bf16 = jnp.float32, jnp.bfloat16


def make(G=2, DEPTH=3, VSPLIT=1, MROWS=8, vmem_mb=100):
    R = G * DH
    NP = H // G
    VR = R // VSPLIT
    assert VR % 128 == 0

    def kern(x_hbm, kt_hbm, vt_hbm, wq_hbm, wo_hbm, wr_hbm, wg_hbm, wu_hbm, wd_hbm, gw_hbm,
             o_ref,
             xs, wrs, gws, wg, wu, wd, wqb, kb, vb, wob, acc_ref,
             sem_s, sem_f, sem_q, sem_k, sem_v, sem_o):

        def cp_q(p, slot):
            return pltpu.make_async_copy(wq_hbm.at[:, pl.ds(pl.multiple_of(p * R, 128), R)], wqb.at[slot], sem_q.at[slot])
        def cp_k(p, slot):
            return pltpu.make_async_copy(kt_hbm.at[pl.ds(pl.multiple_of(p * R, 128), R), pl.ds(SK - WIN, WIN)], kb.at[slot], sem_k.at[slot])
        def cp_v(p, slot, j):
            return pltpu.make_async_copy(vt_hbm.at[pl.ds(pl.multiple_of(p * R + j * VR, 128), VR), pl.ds(SK - WIN, WIN)],
                                         vb.at[slot, pl.ds(j * VR, VR)], sem_v.at[slot, j])
        def cp_o(p, slot):
            return pltpu.make_async_copy(wo_hbm.at[pl.ds(pl.multiple_of(p * R, 128), R), :], wob.at[slot], sem_o.at[slot])

        c_x = pltpu.make_async_copy(x_hbm, xs, sem_s.at[0])
        c_wr = pltpu.make_async_copy(wr_hbm, wrs, sem_s.at[1])
        c_gw = pltpu.make_async_copy(gw_hbm, gws, sem_s.at[2])
        c_g = pltpu.make_async_copy(wg_hbm, wg, sem_f.at[0])
        c_u = pltpu.make_async_copy(wu_hbm, wu, sem_f.at[1])
        c_d = pltpu.make_async_copy(wd_hbm, wd, sem_f.at[2])

        c_g.start(); c_u.start()
        c_x.start(); c_wr.start(); c_gw.start()
        c_d.start()
        for p in range(DEPTH):
            cp_q(p, p).start()
            cp_k(p, p).start()
            cp_o(p, p).start()
            for j in range(VSPLIT):
                cp_v(p, p, j).start()

        c_x.wait(); c_wr.wait(); c_gw.wait()
        xb = xs[0]
        xf = xb.astype(f32)
        xm = jnp.broadcast_to(xb, (MROWS, D))
        gate = jax.nn.sigmoid(jnp.sum(xf * gws[...].astype(f32).reshape(1, D), axis=-1, keepdims=True))
        rsel = jax.nn.sigmoid(jnp.sum(xf * wrs[...].astype(f32).reshape(1, D), axis=-1, keepdims=True))

        c_g.wait()
        hg = jnp.dot(xm, wg[...], preferred_element_type=f32)
        c_u.wait()
        hu = jnp.dot(xm, wu[...], preferred_element_type=f32)
        hh = (hg * jax.nn.sigmoid(hg) * hu).astype(bf16)
        c_d.wait()
        y = jnp.dot(hh, wd[...], preferred_element_type=f32)[:1]
        bres = xf + (xf * 0.0 + y * rsel)
        acc_ref[...] = jnp.zeros_like(acc_ref)

        row = jax.lax.broadcasted_iota(jnp.int32, (MROWS, R), 0)
        col = jax.lax.broadcasted_iota(jnp.int32, (MROWS, R), 1)
        diag = (col >= row * DH) & (col < (row + 1) * DH)

        def body(p, carry):
            slot = p % DEPTH
            nxt = p + DEPTH
            cp_q(p, slot).wait()
            q = jnp.dot(xm, wqb[slot], preferred_element_type=f32)
            qbd = jnp.where(diag, q, 0.0).astype(bf16)
            @pl.when(nxt < NP)
            def _():
                cp_q(nxt, slot).start()
            cp_k(p, slot).wait()
            s = jnp.dot(qbd, kb[slot], preferred_element_type=f32) * (DH ** -0.5)
            @pl.when(nxt < NP)
            def _():
                cp_k(nxt, slot).start()
            m = jnp.max(s, axis=-1, keepdims=True)
            e = jnp.exp(s - m)
            l = jnp.sum(e, axis=-1, keepdims=True)
            pm = e.astype(bf16)
            cp_o(p, slot).wait()
            for j in range(VSPLIT):
                cp_v(p, slot, j).wait()
                r = jax.lax.dot_general(pm, vb[slot, pl.ds(j * VR, VR), :], (((1,), (1,)), ((), ())),
                                        preferred_element_type=f32)
                @pl.when(nxt < NP)
                def _():
                    cp_v(nxt, slot, j).start()
                o = jnp.where(diag[:, j * VR:(j + 1) * VR], r / l, 0.0)
                o = jnp.sum(o, axis=0, keepdims=True)
                ob = jnp.broadcast_to(o.astype(bf16), (MROWS, VR))
                acc_ref[...] += jnp.dot(ob, wob[slot, pl.ds(j * VR, VR), :], preferred_element_type=f32)
            @pl.when(nxt < NP)
            def _():
                cp_o(nxt, slot).start()
            return carry

        jax.lax.fori_loop(0, NP, body, 0)
        a = acc_ref[:1]
        o_ref[0] = (gate * a + (1.0 - gate) * bres).astype(bf16)

    def fn(A_x, A_k_cache, A_v_cache, A_wq, A_wo, B_x, B_w_r, B_w_gate, B_w_up, B_w_down, gate_w):
        kt = jnp.swapaxes(A_k_cache, 2, 3).reshape(H * DH, SK)
        vt = jnp.swapaxes(A_v_cache, 2, 3).reshape(H * DH, SK)
        anyspec = pl.BlockSpec(memory_space=pl.ANY)
        return pl.pallas_call(
            kern,
            in_specs=[anyspec] * 10,
            out_specs=pl.BlockSpec(memory_space=pltpu.VMEM),
            out_shape=jax.ShapeDtypeStruct((1, 1, D), bf16),
            scratch_shapes=[
                pltpu.VMEM((1, 1, D), bf16), pltpu.VMEM((D,), bf16), pltpu.VMEM((D,), bf16),
                pltpu.VMEM((D, F), bf16), pltpu.VMEM((D, F), bf16), pltpu.VMEM((F, D), bf16),
                pltpu.VMEM((DEPTH, D, R), bf16), pltpu.VMEM((DEPTH, R, WIN), bf16),
                pltpu.VMEM((DEPTH, R, WIN), bf16), pltpu.VMEM((DEPTH, R, D), bf16),
                pltpu.VMEM((MROWS, D), f32),
                pltpu.SemaphoreType.DMA((3,)), pltpu.SemaphoreType.DMA((3,)),
                pltpu.SemaphoreType.DMA((DEPTH,)), pltpu.SemaphoreType.DMA((DEPTH,)),
                pltpu.SemaphoreType.DMA((DEPTH, VSPLIT)), pltpu.SemaphoreType.DMA((DEPTH,)),
            ],
            compiler_params=pltpu.CompilerParams(vmem_limit_bytes=vmem_mb * 2**20),
        )(A_x, kt, vt, A_wq, A_wo, B_w_r, B_w_gate, B_w_up, B_w_down, gate_w)
    return fn


_impl = make(G=2, DEPTH=3, VSPLIT=1)


@jax.jit
def pallas_gated_mix__sliding_block_cached__moe_arch_mod__decode_kernel(
    A_x, A_k_cache, A_v_cache, A_wq, A_wo, B_x, B_w_r, B_w_gate, B_w_up, B_w_down, gate_w,
):
    return _impl(A_x, A_k_cache, A_v_cache, A_wq, A_wo, B_x, B_w_r, B_w_gate, B_w_up, B_w_down, gate_w)
```

```python
import jax
import jax.numpy as jnp
import jax.experimental.pallas as pl
import jax.experimental.pallas.tpu as pltpu

H, DH, SK, WIN, D, F = 32, 192, 32768, 4096, 640, 1536
f32, bf16 = jnp.float32, jnp.bfloat16


def make(VSPLIT=3, LN=2048, WROWS=24, MROWS=8, vmem_mb=64, nobc=True, nosc=False, KD=1, prio=True, qsplit=3):
    G = 2
    R = G * DH
    NP = H // G
    VR = R // VSPLIT

    def kern(x_hbm, kt_hbm, vt_hbm, wq_hbm, wo_hbm, wr_hbm, wg_hbm, wu_hbm, wd_hbm, gw_hbm,
             o_ref,
             xs, wrs, gws, wq, wg, wu, wd, wo, kb, vb, qs, acc_ref,
             sems, sem_k, sem_v):
        cnt = [0]

        def issue(src, dst, sem, r_src, c_src, nrows, ncols, drows, dcols):
            for a in range(nrows // drows):
                for b in range(ncols // dcols):
                    rs = r_src + a * drows
                    if not isinstance(rs, int):
                        rs = pl.multiple_of(rs, 8)
                    if dcols == src.shape[1]:
                        s = src.at[pl.ds(rs, drows), :]
                        d = dst.at[pl.ds(a * drows, drows), :]
                    else:
                        s = src.at[pl.ds(rs, drows), pl.ds(c_src + b * dcols, dcols)]
                        d = dst.at[pl.ds(a * drows, drows), pl.ds(b * dcols, dcols)]
                    pltpu.make_async_copy(s, d, sem).start(priority=(cnt[0] % 2) if prio else 0)
                    cnt[0] += 1

        def wait(ref, sem):
            pltpu.make_async_copy(ref, ref, sem).wait()

        def issue_k(p, slot):
            issue(kt_hbm, kb.at[slot], sem_k.at[slot], p * R, SK - WIN, R, WIN, 8, LN)

        def issue_v(p, slot, j):
            issue(vt_hbm, vb.at[slot, pl.ds(j * VR, VR)], sem_v.at[slot, j], p * R + j * VR, SK - WIN, VR, WIN, 8, LN)

        c_x = pltpu.make_async_copy(x_hbm, xs, sems.at[0])
        c_wr = pltpu.make_async_copy(wr_hbm, wrs, sems.at[1])
        c_gw = pltpu.make_async_copy(gw_hbm, gws, sems.at[2])
        c_x.start(); c_wr.start(); c_gw.start()
        S_Q, S_G, S_U, S_D, S_O = 3, 4, 5, 6, 7
        issue(wq_hbm, wq, sems.at[S_Q], 0, 0, D, H * DH, 8, 2048)
        issue(wg_hbm, wg, sems.at[S_G], 0, 0, D, F, 8, F)

        c_x.wait(); c_wr.wait(); c_gw.wait()
        xb = xs[0]
        xf = xb.astype(f32)
        xm = jnp.broadcast_to(xb, (MROWS, D))
        gate = jax.nn.sigmoid(jnp.sum(xf * gws[...].astype(f32).reshape(1, D), axis=-1, keepdims=True))
        rsel = jax.nn.sigmoid(jnp.sum(xf * wrs[...].astype(f32).reshape(1, D), axis=-1, keepdims=True))

        row = jax.lax.broadcasted_iota(jnp.int32, (MROWS, R), 0)
        col = jax.lax.broadcasted_iota(jnp.int32, (MROWS, R), 1)
        diag = (col >= row * DH) & (col < (row + 1) * DH)

        def qblock(c):
            n = H * DH // qsplit
            qs[:, pl.ds(c * n, n)] = jnp.dot(xm, wq[:, pl.ds(c * n, n)], preferred_element_type=f32)

        wait(wq, sems.at[S_Q])
        qblock(0)
        issue(wu_hbm, wu, sems.at[S_U], 0, 0, D, F, 8, F)
        if qsplit > 1: qblock(1)
        issue(wd_hbm, wd, sems.at[S_D], 0, 0, F, D, WROWS, D)
        if qsplit > 2: qblock(2)
        half = H * DH // 2
        issue(wo_hbm, wo.at[pl.ds(0, half)], sems.at[S_O], 0, 0, half, D, WROWS, D)
        wait(wg, sems.at[S_G])
        hg = jnp.dot(xm, wg[...], preferred_element_type=f32)
        issue(wo_hbm, wo.at[pl.ds(half, half)], sems.at[S_O], half, 0, half, D, WROWS, D)
        wait(wu, sems.at[S_U])
        hu = jnp.dot(xm, wu[...], preferred_element_type=f32)
        hh = (hg * jax.nn.sigmoid(hg) * hu).astype(bf16)
        issue_k(0, 0)
        wait(wd, sems.at[S_D])
        y = jnp.dot(hh, wd[...], preferred_element_type=f32)[:1]
        bres = xf + (xf * 0.0 + y * rsel)
        acc_ref[...] = jnp.zeros_like(acc_ref)
        for j in range(VSPLIT):
            issue_v(0, 0, j)
        for d in range(1, KD):
            issue_k(d, d)
            for j in range(VSPLIT):
                issue_v(d, d, j)
        wait(wo, sems.at[S_O])

        def body(p, carry):
            slot = p % KD if KD > 1 else 0
            nxt = p + KD
            q = qs[:, pl.ds(pl.multiple_of(p * R, 128), R)]
            qbd = jnp.where(diag, q, 0.0).astype(bf16)
            wait(kb.at[slot], sem_k.at[slot])
            s = jnp.dot(qbd, kb[slot], preferred_element_type=f32) * (DH ** -0.5)
            @pl.when(nxt < NP)
            def _():
                issue_k(nxt, slot)
            m = jnp.max(s, axis=-1, keepdims=True)
            e = jnp.exp(s - m)
            l = jnp.sum(e, axis=-1, keepdims=True)
            pm = e.astype(bf16)
            for j in range(VSPLIT):
                wait(vb.at[slot, pl.ds(j * VR, VR)], sem_v.at[slot, j])
                r = jax.lax.dot_general(pm, vb[slot, pl.ds(j * VR, VR), :], (((1,), (1,)), ((), ())),
                                        preferred_element_type=f32)
                @pl.when(nxt < NP)
                def _():
                    issue_v(nxt, slot, j)
                o = jnp.where(diag[:, j * VR:(j + 1) * VR], r / l, 0.0)
                o = jnp.sum(o, axis=0, keepdims=True)
                ob = jnp.broadcast_to(o.astype(bf16), (MROWS, VR))
                acc_ref[...] += jnp.dot(ob, wo[pl.ds(pl.multiple_of(p * R + j * VR, 128), VR), :], preferred_element_type=f32)
            return carry

        jax.lax.fori_loop(0, NP, body, 0)
        a = acc_ref[:1]
        o_ref[0] = (gate * a + (1.0 - gate) * bres).astype(bf16)

    def fn(A_x, A_k_cache, A_v_cache, A_wq, A_wo, B_x, B_w_r, B_w_gate, B_w_up, B_w_down, gate_w):
        kt = jnp.swapaxes(A_k_cache, 2, 3).reshape(H * DH, SK)
        vt = jnp.swapaxes(A_v_cache, 2, 3).reshape(H * DH, SK)
        anyspec = pl.BlockSpec(memory_space=pl.ANY)
        return pl.pallas_call(
            kern,
            in_specs=[anyspec] * 10,
            out_specs=pl.BlockSpec(memory_space=pltpu.VMEM),
            out_shape=jax.ShapeDtypeStruct((1, 1, D), bf16),
            scratch_shapes=[
                pltpu.VMEM((1, 1, D), bf16), pltpu.VMEM((D,), bf16), pltpu.VMEM((D,), bf16),
                pltpu.VMEM((D, H * DH), bf16),
                pltpu.VMEM((D, F), bf16), pltpu.VMEM((D, F), bf16), pltpu.VMEM((F, D), bf16),
                pltpu.VMEM((H * DH, D), bf16),
                pltpu.VMEM((KD, R, WIN), bf16), pltpu.VMEM((KD, R, WIN), bf16),
                pltpu.VMEM((MROWS, H * DH), f32),
                pltpu.VMEM((MROWS, D), f32),
                pltpu.SemaphoreType.DMA((8,)), pltpu.SemaphoreType.DMA((KD,)),
                pltpu.SemaphoreType.DMA((KD, VSPLIT)),
            ],
            compiler_params=pltpu.CompilerParams(vmem_limit_bytes=vmem_mb * 2**20, disable_bounds_checks=nobc, disable_semaphore_checks=nosc),
        )(A_x, kt, vt, A_wq, A_wo, B_w_r, B_w_gate, B_w_up, B_w_down, gate_w)
    return fn


_impl = make(WROWS=32, nosc=True)


@jax.jit
def pallas_gated_mix__sliding_block_cached__moe_arch_mod__decode_kernel(
    A_x, A_k_cache, A_v_cache, A_wq, A_wo, B_x, B_w_r, B_w_gate, B_w_up, B_w_down, gate_w,
):
    return _impl(A_x, A_k_cache, A_v_cache, A_wq, A_wo, B_x, B_w_r, B_w_gate, B_w_up, B_w_down, gate_w)
```

```python
import jax
import jax.numpy as jnp
import jax.experimental.pallas as pl
import jax.experimental.pallas.tpu as pltpu

H, DH, SK, WIN, D, F = 32, 192, 32768, 4096, 640, 1536
R = 2 * DH
NP = H // 2
NV = 3
VR = R // NV
M = 8
LN = 2048
WO1 = H * DH - R
f32, bf16 = jnp.float32, jnp.bfloat16


def _dot(a, b):
    return jnp.dot(a, b, preferred_element_type=f32)


def _dot_t(a, b):
    return jax.lax.dot_general(a, b, (((1,), (1,)), ((), ())), preferred_element_type=f32)


def _streams(lst, m):
    per = -(-len(lst) // m)
    return [lst[k * per:(k + 1) * per] for k in range(m)]


def _merge(streams):
    keyed = [((i + 0.5) / len(st), si, d) for si, st in enumerate(streams) for i, d in enumerate(st)]
    keyed.sort(key=lambda t: (t[0], t[1]))
    return [t[2] for t in keyed]


def _kernel(x_hbm, kt_hbm, vt_hbm, wq_hbm, wo_hbm, wr_hbm, wg_hbm, wu_hbm, wd_hbm, gw_hbm,
            o_ref,
            xs, wrs, gws, wq, wg, wu, wd, wo, kb, vb, qs, acc_ref,
            sems, sem_k, sem_v):
    S_X, S_R, S_GW, S_Q, S_G, S_U, S_D, S_O, S_L = range(9)
    cnt = [0]

    def start_all(descs):
        for src, dst, sem in descs:
            pltpu.make_async_copy(src, dst, sem).start(priority=cnt[0] % 2)
            cnt[0] += 1

    def wait(ref, sem):
        pltpu.make_async_copy(ref, ref, sem).wait()

    def w_descs(src, dst, sem, r0, nrows, drows, dcols):
        ncols = src.shape[1]
        assert nrows % drows == 0 and ncols % dcols == 0
        out = []
        for a in range(nrows // drows):
            rows = pl.ds(r0 + a * drows, drows)
            for b in range(ncols // dcols):
                cols = slice(None) if dcols == ncols else pl.ds(b * dcols, dcols)
                out.append((src.at[rows, cols], dst.at[rows, cols], sem))
        return out

    def kv_descs(src, dst, sem, r0, nrows):
        out = []
        for a in range(nrows // 8):
            rs = r0 + a * 8
            if not isinstance(rs, int):
                rs = pl.multiple_of(rs, 8)
            segs = list(range(WIN // LN))
            for b in (segs[::-1] if a % 2 else segs):
                out.append((src.at[pl.ds(rs, 8), pl.ds(SK - WIN + b * LN, LN)],
                            dst.at[pl.ds(a * 8, 8), pl.ds(b * LN, LN)], sem))
        return out

    def issue_k(p):
        start_all(kv_descs(kt_hbm, kb, sem_k, p * R, R))

    def issue_v(p, j):
        start_all(kv_descs(vt_hbm, vb.at[pl.ds(j * VR, VR)], sem_v.at[j], p * R + j * VR, VR))

    c_x = pltpu.make_async_copy(x_hbm, xs, sems.at[S_X])
    c_wr = pltpu.make_async_copy(wr_hbm, wrs, sems.at[S_R])
    c_gw = pltpu.make_async_copy(gw_hbm, gws, sems.at[S_GW])
    c_x.start()
    c_wr.start()
    c_gw.start()
    start_all(_merge(_streams(w_descs(wq_hbm, wq, sems.at[S_Q], 0, D, 8, 2048), 10)))

    st_g = _streams(w_descs(wg_hbm, wg, sems.at[S_G], 0, D, 8, F), 2)
    st_u = _streams(w_descs(wu_hbm, wu, sems.at[S_U], 0, D, 8, F), 2)
    st_d = _streams(w_descs(wd_hbm, wd, sems.at[S_D], 0, F, 16, D), 2)
    st_o = _streams(w_descs(wo_hbm, wo, sems.at[S_O], 0, WO1, 16, D), 6)
    mix = _merge([st[i] for i in range(len(st_o)) for st in (st_g, st_o, st_u, st_d) if i < len(st)])
    n4 = len(mix) // 8 * 2
    start_all(mix[:n4])

    c_x.wait()
    c_wr.wait()
    c_gw.wait()
    xb = xs[0]
    xf = xb.astype(f32)
    xm = jnp.broadcast_to(xb, (M, D))
    gate = jax.nn.sigmoid(jnp.sum(xf * gws[...].astype(f32).reshape(1, D), axis=-1, keepdims=True))
    rsel = jax.nn.sigmoid(jnp.sum(xf * wrs[...].astype(f32).reshape(1, D), axis=-1, keepdims=True))

    def qblock(c):
        n = H * DH // 3
        qs[:, pl.ds(c * n, n)] = _dot(xm, wq[:, pl.ds(c * n, n)])

    wait(wq, sems.at[S_Q])
    qblock(0)
    start_all(mix[n4:2 * n4])
    qblock(1)
    start_all(mix[2 * n4:3 * n4])
    qblock(2)
    start_all(mix[3 * n4:])

    issue_k(0)
    wait(wg, sems.at[S_G])
    hg = _dot(xm, wg[...])
    issue_v(0, 0)
    wait(wu, sems.at[S_U])
    hu = _dot(xm, wu[...])
    hh = (hg * jax.nn.sigmoid(hg) * hu).astype(bf16)
    issue_v(0, 1)
    wait(wd, sems.at[S_D])
    y = _dot(hh, wd[...])[:1]
    issue_v(0, 2)
    bres = xf + (xf * 0.0 + y * rsel)
    acc_ref[...] = jnp.zeros_like(acc_ref)
    wait(wo.at[pl.ds(0, WO1)], sems.at[S_O])

    row = jax.lax.broadcasted_iota(jnp.int32, (M, R), 0)
    col = jax.lax.broadcasted_iota(jnp.int32, (M, R), 1)
    diag = (col >= row * DH) & (col < (row + 1) * DH)

    def body(p, carry):
        nxt = p + 1
        q = qs[:, pl.ds(pl.multiple_of(p * R, 128), R)]
        qbd = jnp.where(diag, q, 0.0).astype(bf16)
        wait(kb, sem_k)
        s = _dot(qbd, kb[...]) * (DH ** -0.5)
        c0 = cnt[0]

        @pl.when(nxt < NP)
        def _():
            issue_k(nxt)

        cnt[0] = c0

        @pl.when(nxt == NP)
        def _():
            start_all(w_descs(wo_hbm, wo, sems.at[S_L], WO1, R, 16, D))

        cnt[0] = c0
        m = jnp.max(s, axis=-1, keepdims=True)
        e = jnp.exp(s - m)
        l = jnp.sum(e, axis=-1, keepdims=True)
        pm = e.astype(bf16)
        outs = []
        for j in range(NV):
            wait(vb.at[pl.ds(j * VR, VR)], sem_v.at[j])
            r = _dot_t(pm, vb[pl.ds(j * VR, VR), :])

            @pl.when(nxt < NP)
            def _():
                issue_v(nxt, j)

            rowj = jax.lax.broadcasted_iota(jnp.int32, (M, VR), 0)
            colj = jax.lax.broadcasted_iota(jnp.int32, (M, VR), 1) + j * VR
            o = jnp.where((colj >= rowj * DH) & (colj < (rowj + 1) * DH), r / l, 0.0)
            o = jnp.sum(o, axis=0, keepdims=True).astype(bf16)
            outs.append(jnp.broadcast_to(o, (M, VR)))
        ob = jnp.concatenate(outs, axis=1)

        @pl.when(nxt == NP)
        def _():
            wait(wo.at[pl.ds(WO1, R)], sems.at[S_L])

        acc_ref[...] += _dot(ob, wo[pl.ds(pl.multiple_of(p * R, 128), R), :])
        return carry

    jax.lax.fori_loop(0, NP, body, 0)
    a = acc_ref[:1]
    o_ref[0] = (gate * a + (1.0 - gate) * bres).astype(bf16)


@jax.jit
def pallas_gated_mix__sliding_block_cached__moe_arch_mod__decode_kernel(
    A_x: jax.Array,
    A_k_cache: jax.Array,
    A_v_cache: jax.Array,
    A_wq: jax.Array,
    A_wo: jax.Array,
    B_x: jax.Array,
    B_w_r: jax.Array,
    B_w_gate: jax.Array,
    B_w_up: jax.Array,
    B_w_down: jax.Array,
    gate_w: jax.Array,
):
    del B_x
    assert A_x.shape == (1, 1, D) and A_k_cache.shape == (1, H, SK, DH)
    kt = jnp.swapaxes(A_k_cache, 2, 3).reshape(H * DH, SK)
    vt = jnp.swapaxes(A_v_cache, 2, 3).reshape(H * DH, SK)
    return pl.pallas_call(
        _kernel,
        in_specs=[pl.BlockSpec(memory_space=pl.ANY)] * 10,
        out_specs=pl.BlockSpec(memory_space=pltpu.VMEM),
        out_shape=jax.ShapeDtypeStruct((1, 1, D), bf16),
        scratch_shapes=[
            pltpu.VMEM((1, 1, D), bf16),
            pltpu.VMEM((D,), bf16),
            pltpu.VMEM((D,), bf16),
            pltpu.VMEM((D, H * DH), bf16),
            pltpu.VMEM((D, F), bf16),
            pltpu.VMEM((D, F), bf16),
            pltpu.VMEM((F, D), bf16),
            pltpu.VMEM((H * DH, D), bf16),
            pltpu.VMEM((R, WIN), bf16),
            pltpu.VMEM((R, WIN), bf16),
            pltpu.VMEM((M, H * DH), f32),
            pltpu.VMEM((M, D), f32),
            pltpu.SemaphoreType.DMA((9,)),
            pltpu.SemaphoreType.DMA(()),
            pltpu.SemaphoreType.DMA((NV,)),
        ],
        compiler_params=pltpu.CompilerParams(
            vmem_limit_bytes=64 * 2**20,
            disable_semaphore_checks=True,
        ),
    )(A_x, kt, vt, A_wq, A_wo, B_w_r, B_w_gate, B_w_up, B_w_down, gate_w)
```
